```python
import os as _os
_os.environ.setdefault("JAX_PLATFORMS", "cpu")
import jax
import jax.numpy as jnp

def _softmax(x, axis=-1):
    return jax.nn.softmax(x, axis=axis)
def _gelu(x):
    return jax.nn.gelu(x, approximate=True)
def _silu(x):
    return jax.nn.silu(x)
def _sigmoid(x):
    return jax.nn.sigmoid(x)
def _layernorm(x, axis=-1, eps=1e-5):
    m = jnp.mean(x, axis=axis, keepdims=True)
    v = jnp.var(x, axis=axis, keepdims=True)
    return (x - m) / jnp.sqrt(v + eps)
def _scatter_add(tgt, idx, src, axis=0):
    return tgt.at[idx].add(src)
def _segment_sum(src, seg, n):
    return jax.ops.segment_sum(src, seg, n)
class _Rng:
    def __init__(self, key):
        self._k = key
    def _next(self):
        self._k, sub = jax.random.split(self._k)
        return sub
    def normal(self, shape):
        return jax.random.normal(self._next(), shape, dtype=jnp.bfloat16)
    def randint(self, lo, hi, shape):
        return jax.random.randint(self._next(), shape, lo, hi, dtype=jnp.int32)
    def uniform(self, shape, lo=0.0, hi=1.0):
        return jax.random.uniform(self._next(), shape, jnp.bfloat16, lo, hi)
    def permutation(self, n):
        return jax.random.permutation(self._next(), n)


kernel_name = 'concat_heads__sliding_block__grouped_kv_mqa__prompt'

def setup_inputs():
    _rng = _Rng(jax.random.key(int.from_bytes(__import__("os").urandom(4), "little")))
    _w = (lambda a: (lambda t: t.astype(jnp.bfloat16) if jnp.issubdtype(t.dtype, jnp.floating) else t)(jnp.asarray(a)))
    def _A_setup():
        B, S, D = 1, 2048, 576
        return {
            "x": _w((lambda *s: _rng.normal(s) * 0.2)(B, S, D)),
            "wqkv": _w((lambda *s: _rng.normal(s) * 0.2)(D, 3 * D)),
            "wo": _w((lambda *s: _rng.normal(s) * 0.05)(D, D)),
        }
    _A_in = _A_setup()

    def _B_setup():
        B, S, D, H = 1, 2048, 576, 32
        Dh = D // H
        return {
            "x": _w((lambda *s: _rng.normal(s) * 0.05)(B, S, D)),
            "wq": _w((lambda *s: _rng.normal(s) * 1.6)(D, H * Dh)),
            "wk": _w((lambda *s: _rng.normal(s) * 1.6)(D, Dh)),
            "wv": _w((lambda *s: _rng.normal(s) * 0.1)(D, Dh)),
            "wo": _w((lambda *s: _rng.normal(s) * 0.1)(H * Dh, D)),
        }
    _B_in = _B_setup()

    return {
        "A_x": _A_in["x"],
        "A_wqkv": _A_in["wqkv"],
        "A_wo": _A_in["wo"],
        "B_x": _B_in["x"],
        "B_wq": _B_in["wq"],
        "B_wk": _B_in["wk"],
        "B_wv": _B_in["wv"],
        "B_wo": _B_in["wo"],
    }

def reference(A_x, A_wqkv, A_wo, B_x, B_wq, B_wk, B_wv, B_wo):
    def _A_ref(x, wqkv, wo):
        B, S, D = x.shape
        H = 32; Dh = D // H; W = 256
        qkv = (lambda x, *d: x.transpose(*d))((x @ wqkv).reshape(B, S, 3, H, Dh), 2, 0, 3, 1, 4)
        q, k, v = qkv[0], qkv[1], qkv[2]
        scores = jnp.einsum("bhqd,bhkd->bhqk", q, k) * (Dh ** -0.5)
        idx = jnp.arange(S)
        mask = (idx[:, None] - idx[None, :] >= 0) & (idx[:, None] - idx[None, :] < W)
        scores = jnp.where(mask[None, None], scores, -1e9)
        p = _softmax(scores, axis=-1)
        o = jnp.einsum("bhqk,bhkd->bhqd", p, v)
        return (lambda x, *d: x.transpose(*d))(o, 0, 2, 1, 3).reshape(B, S, D) @ wo

    def _B_ref(x, wq, wk, wv, wo):
        B, S, D = x.shape
        H = 32
        Dh = D // H
        q = (lambda x, *d: x.transpose(*d))((x @ wq).reshape(B, S, H, Dh), 0, 2, 1, 3)
        k = x @ wk
        v = x @ wv
        scores = jnp.einsum("bhqd,bkd->bhqk", q, k) * (Dh ** -0.5)
        p = _softmax(scores, axis=-1)
        o = jnp.einsum("bhqk,bkd->bhqd", p, v)
        return (lambda x, *d: x.transpose(*d))(o, 0, 2, 1, 3).reshape(B, S, H * Dh) @ wo

    a = _A_ref(A_x, A_wqkv, A_wo)
    b = _B_ref(B_x, B_wq, B_wk, B_wv, B_wo)
    return jnp.concatenate([a, b], axis=-1)
```

```python
import functools
import math

import numpy as np
import jax
import jax.numpy as jnp
import jax.experimental.pallas as pl
import jax.experimental.pallas.tpu as pltpu

S = 2048
D = 576
H = 32
DH = 18
T = 128
NJ = S // T
NEG = -1e30
QSCALE = (DH ** -0.5) * math.log2(math.e)
CH = 512
NCH = S // CH
TPC = CH // T
NBA = 4
QW = 336

f32 = jnp.float32
bf16 = jnp.bfloat16
i32 = jnp.int32

NN = (((1,), (0,)), ((), ()))


def _dot(a, b):
    return jax.lax.dot_general(a, b, NN, preferred_element_type=f32)


def _pack(x):
    return pltpu.bitcast(x, i32)


def _unpack(x):
    return pltpu.bitcast(x, bf16)


def _a_head(h):
    lo = DH * h
    g = lo // T
    if lo + DH <= T * (g + 1):
        return g, 64 * g, lo - T * g
    base = T * g + 112
    return 5 + g, base // 2, lo - base


def _merge4(parts):
    a, b, c, d = parts
    return jnp.concatenate(
        [a[0:16], a[16:24] + b[0:8], b[8:16], b[16:24] + c[0:8], c[8:16],
         c[16:24] + d[0:8], d[8:24]], axis=0)


def _kernel(ax_hbm, wqkv_hbm, awo_hbm, bx_hbm, bwq_hbm, bwkt_hbm, bwvt_hbm, bwo_hbm, out_hbm,
            ax_s, bx_s, wqkv_s, awo_s, bwq_s, bwkt_s, bwvt_s, bwo_s,
            wa_s, wb_s, qta_s, qtb_s, ka_s, vta_s, kb_s, vtb_s, sb_s, sa_s, ota_s, otb_s,
            woa_s, wob_s, out_s, isem, osem):
    def xcopy(hbm, dst, c, k):
        c0 = c * CH if isinstance(c, int) else pl.multiple_of(c * CH, CH)
        return pltpu.make_async_copy(hbm.at[:, pl.ds(c0, CH)], dst.at[c], isem.at[k + c])
    cp_bwq = pltpu.make_async_copy(bwq_hbm, bwq_s, isem.at[0])
    cp_bwk = pltpu.make_async_copy(bwkt_hbm, bwkt_s, isem.at[1])
    cp_bwv = pltpu.make_async_copy(bwvt_hbm, bwvt_s, isem.at[2])
    cp_wqkv = pltpu.make_async_copy(wqkv_hbm, wqkv_s, isem.at[3])
    cp_awo = pltpu.make_async_copy(awo_hbm, awo_s, isem.at[4])
    cp_bwo = pltpu.make_async_copy(bwo_hbm, bwo_s, isem.at[5])
    for cp in ([cp_bwk, cp_bwv, cp_bwq] + [xcopy(bx_hbm, bx_s, c, 6) for c in range(NCH)] + [cp_wqkv]
               + [xcopy(ax_hbm, ax_s, c, 6 + NCH) for c in range(NCH)] + [cp_awo, cp_bwo]):
        cp.start()

    cp_bwk.wait()
    cp_bwv.wait()
    z14 = jnp.zeros((32 - DH, D), bf16)
    wb_s[D:D + 32, :] = jnp.concatenate([bwkt_s[...], z14], axis=0)
    wb_s[D + 32:D + 64, :] = jnp.concatenate([bwvt_s[...], z14], axis=0)
    cp_bwq.wait()
    wb_s[0:D, :] = bwq_s[...].T
    for j in range(NJ):
        qtb_s[j, D // 2:QW, :] = jnp.zeros((QW - D // 2, T), i32)
        qta_s[j, D // 2:QW, :] = jnp.zeros((QW - D // 2, T), i32)

    def bproj(c):
        xcopy(bx_hbm, bx_s, c, 6).wait()
        x = bx_s[c]
        kv = _dot(wb_s[D:D + 64, :], x)
        kt = jnp.concatenate([kv[0:32], jnp.zeros((T - 32, CH), f32)], axis=0)
        k = _pack(kt.astype(bf16).T)
        r0 = c * (CH // 2) if isinstance(c, int) else pl.multiple_of(c * (CH // 2), CH // 2)
        for o in range(8):
            kb_s[o, pl.ds(r0, CH // 2), :] = k if o == 0 else pltpu.roll(k, 2 * o, 1)
        v = kv[32:56].astype(bf16).astype(f32)
        r = jax.lax.broadcasted_iota(i32, (24, CH), 0)
        v = jnp.where(r == DH, 1.0, v)
        for o in range(4):
            vo = v if o == 0 else pltpu.roll(v, 2 * o, 0)
            for t in range(TPC):
                vtb_s[o, c * TPC + t] = vo[:, t * T:(t + 1) * T]
        q = _pack((_dot(wb_s[0:D, :], x) * QSCALE).astype(bf16))
        for t in range(TPC):
            qtb_s[c * TPC + t, 0:D // 2, :] = q[:, t * T:(t + 1) * T]

    def bproj_body(c, _):
        bproj(c)
        return 0
    jax.lax.fori_loop(0, NCH - 1, bproj_body, 0)

    cp_wqkv.wait()
    bproj(NCH - 1)
    for i in range(14):
        n = min(T, 3 * D - T * i)
        wa_s[T * i:T * i + n, :] = wqkv_s[:, T * i:T * i + n].T

    def aproj_body(c, _):
        xcopy(ax_hbm, ax_s, c, 6 + NCH).wait()
        x = ax_s[c]
        kt = jnp.concatenate([_dot(wa_s[D:2 * D, :], x), jnp.zeros((64, CH), f32)], axis=0)
        k = _pack(kt.astype(bf16).T)
        rows = pl.ds(pl.multiple_of(c * (CH // 2), CH // 2), CH // 2)
        for g in range(5):
            ka_s[g, rows, :] = k[:, g * T:(g + 1) * T]
        for g in range(4):
            ka_s[5 + g, rows, :] = k[:, g * T + 112:g * T + 240]
        q = _pack((_dot(wa_s[0:D, :], x) * QSCALE).astype(bf16))
        for t in range(TPC):
            qta_s[c * TPC + t, 0:D // 2, :] = q[:, t * T:(t + 1) * T]
        v = _dot(wa_s[2 * D:3 * D, :], x).astype(bf16).astype(f32)
        for t in range(TPC):
            vta_s[c * TPC + t] = v[:, t * T:(t + 1) * T]
        return 0
    jax.lax.fori_loop(0, NCH, aproj_body, 0)

    rr = jax.lax.broadcasted_iota(i32, (T, T), 0)
    cc = jax.lax.broadcasted_iota(i32, (T, T), 1)

    def b_step(jn, h, hn, buf, m_cur, do_pv=True):
        w0 = 8 * ((9 * hn) // 8)
        ko = (DH * hn - 2 * w0) // 2
        r64 = jax.lax.broadcasted_iota(i32, (64, T), 0)
        qt = _unpack(jnp.where(r64 < 16, qtb_s[jn, w0:w0 + 64, :], 0))
        o = h % 4
        mx = None
        acc = None
        for t in range(NJ):
            if do_pv:
                sc = sb_s[buf, t * T:(t + 1) * T, :]
            s = _dot(_unpack(kb_s[ko, t * 64:(t + 1) * 64, :]), qt)
            sb_s[buf, t * T:(t + 1) * T, :] = s
            mt = jnp.max(s.reshape(T // 8, 8, T), axis=0)
            mx = mt if mx is None else jnp.maximum(mx, mt)
            if do_pv:
                p = jnp.exp2(sc - m_cur).astype(bf16)
                d = _dot(vtb_s[o, t], p)
                acc = d if acc is None else acc + d
        m_new = jnp.max(mx, axis=0, keepdims=True)
        if not do_pv:
            return m_new, None
        dr = (DH + 2 * o) % 24
        inv = 1.0 / acc[dr:dr + 1, :]
        r = jax.lax.broadcasted_iota(i32, (24, T), 0)
        res = jnp.where((r >= 2 * o) & (r < 2 * o + DH), acc * inv, 0.0)
        return m_new, res

    ms = tuple(b_step(0, 0, u, u, None, do_pv=False)[0] for u in range(2))

    def b_body(j, ms):
        ms = list(ms)
        jn1 = jnp.minimum(j + 1, NJ - 1)
        parts = []
        for h in range(H):
            hn = (h + 2) % H
            jn = j if h + 2 < H else jn1
            ms[h % 2], res = b_step(jn, h, hn, h % 2, ms[h % 2])
            parts.append(res)
            if h % 4 == 3:
                G = h // 4
                otb_s[j, 72 * G:72 * G + 72, :] = _merge4(parts)
                parts = []
        return tuple(ms)
    jax.lax.fori_loop(0, NJ, b_body, ms)

    cp_awo.wait()
    cp_bwo.wait()
    woa_s[...] = awo_s[...].T
    wob_s[...] = bwo_s[...].T

    def unit(j, first):
        return (j, first)

    tri = cc >= rr

    def a_step(cur, h, nxt, hn, buf, m_cur):
        slab, w0, qo = _a_head(hn)
        R = 8 * ((DH * h) // 8)
        o = DH * h - R
        dr = (o + DH) % 24
        r24 = jax.lax.broadcasted_iota(i32, (24, T), 0)
        vmask = (r24 >= o) & (r24 < o + DH)
        r64 = jax.lax.broadcasted_iota(i32, (64, T), 0)
        qmask = (r64 >= qo // 2) & (r64 < qo // 2 + 9)

        def scores(jq, kt):
            q = _unpack(jnp.where(qmask, qta_s[jq, w0:w0 + 64, :], 0))
            k0 = kt * 64 if isinstance(kt, int) else pl.multiple_of(kt * 64, 64)
            return _dot(_unpack(ka_s[slab, pl.ds(k0, 64), :]), q)

        def colmax(s):
            return jnp.max(s.reshape(T // 8, 8, T), axis=0)

        def pv(kt, p):
            vt = jnp.where(vmask, vta_s[kt, R:R + 24, :], jnp.where(r24 == dr, 1.0, 0.0))
            return _dot(vt, p.astype(bf16))

        def finish(a):
            return jnp.where(vmask, a * (1.0 / a[dr:dr + 1, :]), 0.0)

        sc = None
        if cur is not None:
            n = 3 if cur[1] else 2
            sc = [sa_s[buf, s * T:(s + 1) * T, :] for s in range(n)]
        jn, first_n = nxt
        if first_n:
            new = [jnp.where(tri, scores(0, 0), NEG), scores(1, 0), jnp.where(tri, scores(1, 1), NEG)]
            mx = [colmax(new[0]), jnp.maximum(colmax(new[1]), colmax(new[2]))]
        else:
            new = [jnp.where(tri, scores(jn, jn), scores(jn, jn - 2)), scores(jn, jn - 1)]
            mx = [jnp.maximum(colmax(new[0]), colmax(new[1]))]
        for s, v in enumerate(new):
            sa_s[buf, s * T:(s + 1) * T, :] = v
        m_new = [jnp.max(m, axis=0, keepdims=True) for m in mx]
        if cur is None:
            return m_new, None
        j, first = cur
        if first:
            res = [finish(pv(0, jnp.exp2(sc[0] - m_cur[0]))),
                   finish(pv(0, jnp.exp2(sc[1] - m_cur[1])) + pv(1, jnp.exp2(sc[2] - m_cur[1])))]
        else:
            pm = jnp.exp2(sc[0] - m_cur[0])
            res = [finish(pv(j, jnp.where(tri, pm, 0.0)) + pv(j - 2, jnp.where(tri, 0.0, pm))
                          + pv(j - 1, jnp.exp2(sc[1] - m_cur[0])))]
        return m_new, res

    def out_tile(j):
        ra = _dot(woa_s[...], ota_s[j].astype(bf16))
        rb = _dot(wob_s[...], otb_s[j].astype(bf16))
        out_s[j] = jnp.concatenate([ra.astype(bf16), rb.astype(bf16)], axis=0).T
        r0 = j * T if isinstance(j, int) else pl.multiple_of(j * T, T)
        pltpu.make_async_copy(out_s.at[j], out_hbm.at[pl.ds(r0, T), :], osem.at[j]).start()

    def a_sweep(cur_fn, nxt_fn, ms):
        jq0 = cur_fn(0)[0]
        ms = list(ms)
        parts = None
        for h in range(H):
            hn = (h + NBA) % H
            ms[h % NBA], res = a_step(cur_fn(h), h, nxt_fn(h), hn, h % NBA, ms[h % NBA])
            parts = [[r] for r in res] if h % 4 == 0 else [p + [r] for p, r in zip(parts, res)]
            if h % 4 == 3:
                G = h // 4
                for gi, p in enumerate(parts):
                    ota_s[jq0 + gi, 72 * G:72 * G + 72, :] = _merge4(p)
        return ms

    ms = [a_step(None, 0, unit(0, True), u, u, None)[0] for u in range(NBA)]
    ms = a_sweep(lambda h: unit(0, True),
                 lambda h: unit(0, True) if h + NBA < H else unit(2, False), ms)
    out_tile(0)

    def a_body(j, ms):
        jn1 = jnp.minimum(j + 1, NJ - 1)
        out_tile(j - 1)
        ms = a_sweep(lambda h: unit(j, False),
                     lambda h: unit(j if h + NBA < H else jn1, False), [list(m) for m in ms])
        return tuple(tuple(m) for m in ms)
    jax.lax.fori_loop(2, NJ, a_body, tuple(tuple(m) for m in ms))
    out_tile(NJ - 1)

    for j in range(NJ):
        pltpu.make_async_copy(out_s.at[j], out_hbm.at[pl.ds(j * T, T), :], osem.at[j]).wait()


@jax.jit
def pallas_concat_heads__sliding_block__grouped_kv_mqa__prompt_kernel(
    A_x: jax.Array,
    A_wqkv: jax.Array,
    A_wo: jax.Array,
    B_x: jax.Array,
    B_wq: jax.Array,
    B_wk: jax.Array,
    B_wv: jax.Array,
    B_wo: jax.Array,
):
    scratch = [
        pltpu.VMEM((NCH, D, CH), bf16),
        pltpu.VMEM((NCH, D, CH), bf16),
        pltpu.VMEM((D, 3 * D), bf16),
        pltpu.VMEM((D, D), bf16),
        pltpu.VMEM((D, D), bf16),
        pltpu.VMEM((DH, D), bf16),
        pltpu.VMEM((DH, D), bf16),
        pltpu.VMEM((D, D), bf16),
        pltpu.VMEM((3 * D, D), bf16),
        pltpu.VMEM((D + 64, D), bf16),
        pltpu.VMEM((NJ, QW, T), i32),
        pltpu.VMEM((NJ, QW, T), i32),
        pltpu.VMEM((9, S // 2, T), i32),
        pltpu.VMEM((NJ, D, T), f32),
        pltpu.VMEM((8, S // 2, T), i32),
        pltpu.VMEM((4, NJ, 24, T), f32),
        pltpu.VMEM((2, S, T), f32),
        pltpu.VMEM((NBA, 3 * T, T), f32),
        pltpu.VMEM((NJ, D, T), f32),
        pltpu.VMEM((NJ, D, T), f32),
        pltpu.VMEM((D, D), bf16),
        pltpu.VMEM((D, D), bf16),
        pltpu.VMEM((NJ, T, 2 * D), bf16),
        pltpu.SemaphoreType.DMA((6 + 2 * NCH,)),
        pltpu.SemaphoreType.DMA((NJ,)),
    ]
    anyspec = pl.BlockSpec(memory_space=pl.ANY)
    out = pl.pallas_call(
        _kernel,
        out_shape=jax.ShapeDtypeStruct((S, 2 * D), bf16),
        in_specs=[anyspec] * 8,
        out_specs=anyspec,
        scratch_shapes=scratch,
        compiler_params=pltpu.CompilerParams(vmem_limit_bytes=100 * 1024 * 1024),
        name="fused_attn_pair",
    )(A_x.reshape(S, D).T, A_wqkv, A_wo, B_x.reshape(S, D).T, B_wq, B_wk.T, B_wv.T, B_wo)
    return out.reshape(1, S, 2 * D)
```

```python
import functools
import math

import numpy as np
import jax
import jax.numpy as jnp
import jax.experimental.pallas as pl
import jax.experimental.pallas.tpu as pltpu

S = 2048
D = 576
H = 32
DH = 18
T = 128
NJ = S // T
NEG = -1e30
QSCALE = (DH ** -0.5) * math.log2(math.e)
CH = 512
NCH = S // CH
TPC = CH // T
NBA = 4
QW = 336

f32 = jnp.float32
bf16 = jnp.bfloat16
i32 = jnp.int32

NN = (((1,), (0,)), ((), ()))


def _dot(a, b):
    return jax.lax.dot_general(a, b, NN, preferred_element_type=f32)


def _pack(x):
    return pltpu.bitcast(x, i32)


def _unpack(x):
    return pltpu.bitcast(x, bf16)


def _merge4(parts):
    a, b, c, d = parts
    return jnp.concatenate(
        [a[0:16], a[16:24] + b[0:8], b[8:16], b[16:24] + c[0:8], c[8:16],
         c[16:24] + d[0:8], d[8:24]], axis=0)


def _kernel(ax_hbm, wqkv_hbm, awo_hbm, bx_hbm, bwq_hbm, bwkt_hbm, bwvt_hbm, bwo_hbm, out_hbm,
            ax_s, bx_s, wqkv_s, awo_s, bwq_s, bwkt_s, bwvt_s, bwo_s,
            wa_s, wb_s, qta_s, qtb_s, ka_s, vta_s, kb_s, vtb_s, sb_s, sa_s, ota_s, otb_s,
            woa_s, wob_s, out_s, carry_s, bias_s, isem, osem):
    def xcopy(hbm, dst, c, k):
        c0 = c * CH if isinstance(c, int) else pl.multiple_of(c * CH, CH)
        return pltpu.make_async_copy(hbm.at[:, pl.ds(c0, CH)], dst.at[c], isem.at[k + c])
    cp_bwq = pltpu.make_async_copy(bwq_hbm, bwq_s, isem.at[0])
    cp_bwk = pltpu.make_async_copy(bwkt_hbm, bwkt_s, isem.at[1])
    cp_bwv = pltpu.make_async_copy(bwvt_hbm, bwvt_s, isem.at[2])
    cp_wqkv = pltpu.make_async_copy(wqkv_hbm, wqkv_s, isem.at[3])
    cp_awo = pltpu.make_async_copy(awo_hbm, awo_s, isem.at[4])
    cp_bwo = pltpu.make_async_copy(bwo_hbm, bwo_s, isem.at[5])
    for cp in ([cp_bwk, cp_bwv, cp_bwq] + [xcopy(bx_hbm, bx_s, c, 6) for c in range(NCH)] + [cp_wqkv]
               + [xcopy(ax_hbm, ax_s, c, 6 + NCH) for c in range(NCH)] + [cp_awo, cp_bwo]):
        cp.start()

    cp_bwk.wait()
    cp_bwv.wait()
    z14 = jnp.zeros((32 - DH, D), bf16)
    wb_s[D:D + 32, :] = jnp.concatenate([bwkt_s[...], z14], axis=0)
    wb_s[D + 32:D + 64, :] = jnp.concatenate([bwvt_s[...], z14], axis=0)
    cp_bwq.wait()
    wb_s[0:D, :] = bwq_s[...].T
    for j in range(NJ):
        qtb_s[j, D // 2:QW, :] = jnp.zeros((QW - D // 2, T), i32)

    def bproj(c):
        xcopy(bx_hbm, bx_s, c, 6).wait()
        x = bx_s[c]
        kv = _dot(wb_s[D:D + 64, :], x)
        kt = jnp.concatenate([kv[0:32], jnp.zeros((T - 32, CH), f32)], axis=0)
        k = _pack(kt.astype(bf16).T)
        r0 = c * (CH // 2) if isinstance(c, int) else pl.multiple_of(c * (CH // 2), CH // 2)
        for o in range(8):
            kb_s[o, pl.ds(r0, CH // 2), :] = k if o == 0 else pltpu.roll(k, 2 * o, 1)
        v = kv[32:56].astype(bf16).astype(f32)
        r = jax.lax.broadcasted_iota(i32, (24, CH), 0)
        v = jnp.where(r == DH, 1.0, v)
        for o in range(4):
            vo = v if o == 0 else pltpu.roll(v, 2 * o, 0)
            for t in range(TPC):
                vtb_s[o, c * TPC + t] = vo[:, t * T:(t + 1) * T]
        q = _pack((_dot(wb_s[0:D, :], x) * QSCALE).astype(bf16))
        for t in range(TPC):
            qtb_s[c * TPC + t, 0:D // 2, :] = q[:, t * T:(t + 1) * T]

    def bproj_body(c, _):
        bproj(c)
        return 0
    jax.lax.fori_loop(0, NCH - 1, bproj_body, 0)

    cp_wqkv.wait()
    bproj(NCH - 1)
    for i in range(14):
        n = min(T, 3 * D - T * i)
        wa_s[T * i:T * i + n, :] = wqkv_s[:, T * i:T * i + n].T

    def aproj_body(c, _):
        xcopy(ax_hbm, ax_s, c, 6 + NCH).wait()
        x = ax_s[c]
        kt = _dot(wa_s[D:2 * D, :], x).astype(bf16)
        rows = pl.ds(pl.multiple_of(c * (CH // 2), CH // 2), CH // 2)
        lane = jax.lax.broadcasted_iota(i32, (CH // 2, T), 1)
        for h in range(H):
            base = 16 * ((DH * h) // 16)
            w = kt[base:base + 32]
            w = _pack(jnp.concatenate([w, w, w, w], axis=0).T)
            ext = jnp.concatenate([carry_s[h], w], axis=0)
            carry_s[h] = w[CH // 2 - 48:]
            n = CH // 2
            ka_s[h, rows, :] = jnp.where(
                lane < 64, jnp.where(lane < 32, ext[0:n], ext[16:n + 16]),
                jnp.where(lane < 96, ext[32:n + 32], ext[48:n + 48]))
        q = _pack((_dot(wa_s[0:D, :], x) * QSCALE).astype(bf16))
        r16 = jax.lax.broadcasted_iota(i32, (16, CH), 0)
        for h in range(H):
            base = 16 * ((DH * h) // 16)
            qo = (DH * h - base) // 2
            w = jnp.where((r16 >= qo) & (r16 < qo + 9), q[base // 2:base // 2 + 16], 0)
            for t in range(TPC):
                qta_s[c * TPC + t, h] = w[:, t * T:(t + 1) * T]
        v = _dot(wa_s[2 * D:3 * D, :], x).astype(bf16).astype(f32)
        r24 = jax.lax.broadcasted_iota(i32, (24, CH), 0)
        for h in range(H):
            R = 8 * ((DH * h) // 8)
            o = DH * h - R
            w = jnp.where((r24 >= o) & (r24 < o + DH), v[R:R + 24],
                          jnp.where(r24 == (o + DH) % 24, 1.0, 0.0))
            for t in range(TPC):
                vta_s[c * TPC + t, h] = w[:, t * T:(t + 1) * T]
        return 0
    carry_s[...] = jnp.zeros(carry_s.shape, i32)
    jax.lax.fori_loop(0, NCH, aproj_body, 0)

    rr = jax.lax.broadcasted_iota(i32, (T, T), 0)
    cc = jax.lax.broadcasted_iota(i32, (T, T), 1)

    def b_step(jn, h, hn, buf, m_cur, do_pv=True):
        w0 = 8 * ((9 * hn) // 8)
        ko = (DH * hn - 2 * w0) // 2
        r64 = jax.lax.broadcasted_iota(i32, (64, T), 0)
        qt = _unpack(jnp.where(r64 < 16, qtb_s[jn, w0:w0 + 64, :], 0))
        o = h % 4
        mx = None
        acc = None
        for t in range(NJ):
            if do_pv:
                sc = sb_s[buf, t * T:(t + 1) * T, :]
            s = _dot(_unpack(kb_s[ko, t * 64:(t + 1) * 64, :]), qt)
            sb_s[buf, t * T:(t + 1) * T, :] = s
            mt = jnp.max(s.reshape(T // 8, 8, T), axis=0)
            mx = mt if mx is None else jnp.maximum(mx, mt)
            if do_pv:
                p = jnp.exp2(sc - m_cur).astype(bf16)
                d = _dot(vtb_s[o, t], p)
                acc = d if acc is None else acc + d
        m_new = jnp.max(mx, axis=0, keepdims=True)
        if not do_pv:
            return m_new, None
        dr = (DH + 2 * o) % 24
        inv = 1.0 / acc[dr:dr + 1, :]
        r = jax.lax.broadcasted_iota(i32, (24, T), 0)
        res = jnp.where((r >= 2 * o) & (r < 2 * o + DH), acc * inv, 0.0)
        return m_new, res

    ms = tuple(b_step(0, 0, u, u, None, do_pv=False)[0] for u in range(2))

    def b_body(j, ms):
        ms = list(ms)
        jn1 = jnp.minimum(j + 1, NJ - 1)
        parts = []
        for h in range(H):
            hn = (h + 2) % H
            jn = j if h + 2 < H else jn1
            ms[h % 2], res = b_step(jn, h, hn, h % 2, ms[h % 2])
            parts.append(res)
            if h % 4 == 3:
                G = h // 4
                otb_s[j, 72 * G:72 * G + 72, :] = _merge4(parts)
                parts = []
        return tuple(ms)
    jax.lax.fori_loop(0, NJ, b_body, ms)

    cp_awo.wait()
    cp_bwo.wait()
    woa_s[...] = awo_s[...].T
    wob_s[...] = bwo_s[...].T

    def unit(j, first):
        return (j, first)

    bias_s[0:T, :] = jnp.where(cc >= rr, 0.0, NEG)
    bias_s[T:T + 32, :] = jnp.where(rr > (cc & 31), 0.0, NEG)[0:32]
    bias_s[T + 32:T + 64, :] = jnp.where(rr <= (cc & 31), 0.0, NEG)[0:32]

    def a_step(cur, h, nxt, hn, buf, m_cur):
        o = DH * h - 8 * ((DH * h) // 8)
        dr = (o + DH) % 24
        l16 = jax.lax.broadcasted_iota(i32, (16, T), 1)
        l8 = jax.lax.broadcasted_iota(i32, (8, T), 1)

        def krows(w0, n):
            w0 = w0 if isinstance(w0, int) else pl.multiple_of(w0, 8)
            return ka_s[hn, pl.ds(w0, n), :]

        def plain_scores(jq, kt):
            q = jnp.concatenate([jnp.zeros((48, T), i32), qta_s[jq, hn]], axis=0)
            return _dot(_unpack(krows(kt * 64, 64)), _unpack(q))

        def by_group(srcs):
            out = srcs[3]
            for g in (2, 1, 0):
                if srcs[g] is None and out is None:
                    continue
                out = jnp.where(l8 < 32 * (g + 1), 0 if srcs[g] is None else srcs[g],
                                0 if out is None else out)
            return out

        def sheared_scores(jq):
            w = qta_s[jq, hn]
            q = jnp.concatenate(
                [jnp.where(l16 < 32, w, 0), jnp.where(l16 < 32, 0, jnp.where(l16 < 64, w, 0)),
                 jnp.where(l16 < 64, 0, jnp.where(l16 < 96, w, 0)), jnp.where(l16 < 96, 0, w)], axis=0)
            lo = krows((jq - 2) * 64 + 48, 64)
            hi = krows((jq - 1) * 64 + 48 + 16, 64)
            blocks = [lo[0:16]]
            for b in range(2, 8):
                blocks.append(jnp.where(l8 < 32 * ((7 - b) // 2 + 1), lo[8 * b:8 * b + 8], hi[8 * b - 16:8 * b - 8]))
            blocks.append(hi[48:64])
            s = _dot(_unpack(jnp.concatenate(blocks, axis=0)), _unpack(q))
            return jnp.concatenate([s[0:32] + bias_s[T:T + 32, :], s[32:128],
                                    s[128:160] + bias_s[T + 32:T + 64, :]], axis=0)

        def colmax(s):
            return jnp.max(s.reshape(s.shape[0] // 8, 8, T), axis=0)

        def pv(kt, p):
            return _dot(vta_s[kt, h], p)

        def finish(a):
            a = a * (1.0 / a[dr:dr + 1, :])
            b0 = 8 * (dr // 8)
            r8 = jax.lax.broadcasted_iota(i32, (8, T), 0)
            blk = jnp.where(r8 == dr - b0, 0.0, a[b0:b0 + 8])
            return jnp.concatenate([p for p in (a[0:b0], blk, a[b0 + 8:24]) if p.shape[0]], axis=0)

        def prob(s, m):
            return jnp.exp2(s - m).astype(bf16)

        sc = None
        if cur is not None:
            sizes = (T, T, T) if cur[1] else (160, T)
            sc, r0 = [], 0
            for n in sizes:
                sc.append(sa_s[buf, r0:r0 + n, :])
                r0 += n
        jn, first_n = nxt
        if first_n:
            new = [plain_scores(0, 0) + bias_s[0:T, :], plain_scores(1, 0),
                   plain_scores(1, 1) + bias_s[0:T, :]]
            mx = [colmax(new[0]), jnp.maximum(colmax(new[1]), colmax(new[2]))]
        else:
            new = [sheared_scores(jn), plain_scores(jn, jn - 1)]
            mx = [jnp.maximum(colmax(new[0]), colmax(new[1]))]
        r0 = 0
        for v in new:
            sa_s[buf, r0:r0 + v.shape[0], :] = v
            r0 += v.shape[0]
        m_new = [jnp.max(m, axis=0, keepdims=True) for m in mx]
        if cur is None:
            return m_new, None
        j, first = cur
        if first:
            res = [finish(pv(0, prob(sc[0], m_cur[0]))),
                   finish(pv(0, prob(sc[1], m_cur[1])) + pv(1, prob(sc[2], m_cur[1])))]
        else:
            pw = _pack(prob(sc[0], m_cur[0]))
            pb = [pw[8 * b:8 * b + 8] for b in range(10)]
            trail = jnp.concatenate(
                [by_group([pb[b - 2 * g] if b >= 2 * g else None for g in range(4)]) for b in range(8)],
                axis=0)
            diag = jnp.concatenate(
                [by_group([pb[b + 8 - 2 * g] if b < 2 * (g + 1) else None for g in range(4)])
                 for b in range(8)], axis=0)
            res = [finish(pv(j, _unpack(diag)) + pv(j - 2, _unpack(trail))
                          + pv(j - 1, prob(sc[1], m_cur[0])))]
        return m_new, res

    def out_tile(j):
        ra = _dot(woa_s[...], ota_s[j].astype(bf16))
        rb = _dot(wob_s[...], otb_s[j].astype(bf16))
        out_s[j] = jnp.concatenate([ra.astype(bf16), rb.astype(bf16)], axis=0).T
        r0 = j * T if isinstance(j, int) else pl.multiple_of(j * T, T)
        pltpu.make_async_copy(out_s.at[j], out_hbm.at[pl.ds(r0, T), :], osem.at[j]).start()

    def a_sweep(cur_fn, nxt_fn, ms):
        jq0 = cur_fn(0)[0]
        ms = list(ms)
        parts = None
        for h in range(H):
            hn = (h + NBA) % H
            ms[h % NBA], res = a_step(cur_fn(h), h, nxt_fn(h), hn, h % NBA, ms[h % NBA])
            parts = [[r] for r in res] if h % 4 == 0 else [p + [r] for p, r in zip(parts, res)]
            if h % 4 == 3:
                G = h // 4
                for gi, p in enumerate(parts):
                    ota_s[jq0 + gi, 72 * G:72 * G + 72, :] = _merge4(p)
        return ms

    ms = [a_step(None, 0, unit(0, True), u, u, None)[0] for u in range(NBA)]
    ms = a_sweep(lambda h: unit(0, True),
                 lambda h: unit(0, True) if h + NBA < H else unit(2, False), ms)
    out_tile(0)

    def a_body(j, ms):
        jn1 = jnp.minimum(j + 1, NJ - 1)
        out_tile(j - 1)
        ms = a_sweep(lambda h: unit(j, False),
                     lambda h: unit(j if h + NBA < H else jn1, False), [list(m) for m in ms])
        return tuple(tuple(m) for m in ms)
    jax.lax.fori_loop(2, NJ, a_body, tuple(tuple(m) for m in ms))
    out_tile(NJ - 1)

    for j in range(NJ):
        pltpu.make_async_copy(out_s.at[j], out_hbm.at[pl.ds(j * T, T), :], osem.at[j]).wait()


@jax.jit
def pallas_concat_heads__sliding_block__grouped_kv_mqa__prompt_kernel(
    A_x: jax.Array,
    A_wqkv: jax.Array,
    A_wo: jax.Array,
    B_x: jax.Array,
    B_wq: jax.Array,
    B_wk: jax.Array,
    B_wv: jax.Array,
    B_wo: jax.Array,
):
    scratch = [
        pltpu.VMEM((NCH, D, CH), bf16),
        pltpu.VMEM((NCH, D, CH), bf16),
        pltpu.VMEM((D, 3 * D), bf16),
        pltpu.VMEM((D, D), bf16),
        pltpu.VMEM((D, D), bf16),
        pltpu.VMEM((DH, D), bf16),
        pltpu.VMEM((DH, D), bf16),
        pltpu.VMEM((D, D), bf16),
        pltpu.VMEM((3 * D, D), bf16),
        pltpu.VMEM((D + 64, D), bf16),
        pltpu.VMEM((NJ, H, 16, T), i32),
        pltpu.VMEM((NJ, QW, T), i32),
        pltpu.VMEM((H, S // 2, T), i32),
        pltpu.VMEM((NJ, H, 24, T), f32),
        pltpu.VMEM((8, S // 2, T), i32),
        pltpu.VMEM((4, NJ, 24, T), f32),
        pltpu.VMEM((2, S, T), f32),
        pltpu.VMEM((NBA, 3 * T, T), f32),
        pltpu.VMEM((NJ, D, T), f32),
        pltpu.VMEM((NJ, D, T), f32),
        pltpu.VMEM((D, D), bf16),
        pltpu.VMEM((D, D), bf16),
        pltpu.VMEM((NJ, T, 2 * D), bf16),
        pltpu.VMEM((H, 48, T), i32),
        pltpu.VMEM((T + 64, T), f32),
        pltpu.SemaphoreType.DMA((6 + 2 * NCH,)),
        pltpu.SemaphoreType.DMA((NJ,)),
    ]
    anyspec = pl.BlockSpec(memory_space=pl.ANY)
    out = pl.pallas_call(
        _kernel,
        out_shape=jax.ShapeDtypeStruct((S, 2 * D), bf16),
        in_specs=[anyspec] * 8,
        out_specs=anyspec,
        scratch_shapes=scratch,
        compiler_params=pltpu.CompilerParams(vmem_limit_bytes=100 * 1024 * 1024),
        name="fused_attn_pair",
    )(A_x.reshape(S, D).T, A_wqkv, A_wo, B_x.reshape(S, D).T, B_wq, B_wk.T, B_wv.T, B_wo)
    return out.reshape(1, S, 2 * D)
```

```python
import math

import jax
import jax.numpy as jnp
import jax.experimental.pallas as pl
import jax.experimental.pallas.tpu as pltpu

S = 2048
D = 576
H = 32
DH = 18
T = 128
NJ = S // T
NEG = -1e30
QSCALE = (DH ** -0.5) * math.log2(math.e)
CH = 512
NCH = S // CH
TPC = CH // T
NBA = 4
NVV = 14
NACC = 7
RV = 8 * NVV
V0 = S - RV
QW = 336

f32 = jnp.float32
bf16 = jnp.bfloat16
i32 = jnp.int32

NN = (((1,), (0,)), ((), ()))


def _dot(a, b):
    return jax.lax.dot_general(a, b, NN, preferred_element_type=f32)


def _pack(x):
    return pltpu.bitcast(x, i32)


def _unpack(x):
    return pltpu.bitcast(x, bf16)


def _merge4(parts):
    a, b, c, d = parts
    return jnp.concatenate(
        [a[0:16], a[16:24] + b[0:8], b[8:16], b[16:24] + c[0:8], c[8:16],
         c[16:24] + d[0:8], d[8:24]], axis=0)


def _kernel(ax_hbm, wqkv_hbm, awo_hbm, bx_hbm, bwq_hbm, bwkt_hbm, bwvt_hbm, bwo_hbm, out_hbm,
            ax_s, bx_s, wqkv_s, awo_s, bwq_s, bwkt_s, bwvt_s, bwo_s,
            wa_s, wb_s, qta_s, qtb_s, ka_s, vta_s, kb_s, vtb_s, sb_s, sa_s, ota_s, otb_s,
            woa_s, wob_s, out_s, carry_s, bias_s, qf_s, kbc_s, vb_s, z_s, isem, osem):
    def xcopy(hbm, dst, c, k):
        c0 = c * CH if isinstance(c, int) else pl.multiple_of(c * CH, CH)
        return pltpu.make_async_copy(hbm.at[:, pl.ds(c0, CH)], dst.at[c], isem.at[k + c])
    cp_bwq = pltpu.make_async_copy(bwq_hbm, bwq_s, isem.at[0])
    cp_bwk = pltpu.make_async_copy(bwkt_hbm, bwkt_s, isem.at[1])
    cp_bwv = pltpu.make_async_copy(bwvt_hbm, bwvt_s, isem.at[2])
    cp_wqkv = pltpu.make_async_copy(wqkv_hbm, wqkv_s, isem.at[3])
    cp_awo = pltpu.make_async_copy(awo_hbm, awo_s, isem.at[4])
    cp_bwo = pltpu.make_async_copy(bwo_hbm, bwo_s, isem.at[5])
    for cp in ([cp_bwk, cp_bwv, cp_bwq] + [xcopy(bx_hbm, bx_s, c, 6) for c in range(NCH)] + [cp_wqkv]
               + [xcopy(ax_hbm, ax_s, c, 6 + NCH) for c in range(NCH)] + [cp_awo, cp_bwo]):
        cp.start()

    cp_bwk.wait()
    cp_bwv.wait()
    z14 = jnp.zeros((32 - DH, D), bf16)
    wb_s[D:D + 32, :] = jnp.concatenate([bwkt_s[...], z14], axis=0)
    wb_s[D + 32:D + 64, :] = jnp.concatenate([bwvt_s[...], z14], axis=0)
    cp_bwq.wait()
    wb_s[0:D, :] = bwq_s[...].T
    for j in range(NJ):
        qtb_s[j, D // 2:QW, :] = jnp.zeros((QW - D // 2, T), i32)

    def bproj(c):
        xcopy(bx_hbm, bx_s, c, 6).wait()
        x = bx_s[c]
        kv = _dot(wb_s[D:D + 64, :], x)
        kt = jnp.concatenate([kv[0:32], jnp.zeros((T - 32, CH), f32)], axis=0)
        k = _pack(kt.astype(bf16).T)
        r0 = c * (CH // 2) if isinstance(c, int) else pl.multiple_of(c * (CH // 2), CH // 2)
        for o in range(8):
            kb_s[o, pl.ds(r0, CH // 2), :] = k if o == 0 else pltpu.roll(k, 2 * o, 1)
        v = kv[32:56].astype(bf16).astype(f32)
        r = jax.lax.broadcasted_iota(i32, (24, CH), 0)
        v = jnp.where(r == DH, 1.0, v)
        for o in range(4):
            vo = v if o == 0 else pltpu.roll(v, 2 * o, 0)
            for t in range(TPC):
                vtb_s[o, c * TPC + t] = vo[:, t * T:(t + 1) * T]
        qb = (_dot(wb_s[0:D, :], x) * QSCALE).astype(bf16)
        q = _pack(qb)
        qb = qb.astype(f32)
        for t in range(TPC):
            qtb_s[c * TPC + t, 0:D // 2, :] = q[:, t * T:(t + 1) * T]
            qf_s[c * TPC + t] = qb[:, t * T:(t + 1) * T]

    def bproj_body(c, _):
        bproj(c)
        return 0
    jax.lax.fori_loop(0, NCH - 1, bproj_body, 0)

    cp_wqkv.wait()
    bproj(NCH - 1)
    for i in range(14):
        n = min(T, 3 * D - T * i)
        wa_s[T * i:T * i + n, :] = wqkv_s[:, T * i:T * i + n].T

    def aproj_body(c, _):
        xcopy(ax_hbm, ax_s, c, 6 + NCH).wait()
        x = ax_s[c]
        kt = _dot(wa_s[D:2 * D, :], x).astype(bf16)
        rows = pl.ds(pl.multiple_of(c * (CH // 2), CH // 2), CH // 2)
        lane = jax.lax.broadcasted_iota(i32, (CH // 2, T), 1)
        for h in range(H):
            base = 16 * ((DH * h) // 16)
            w = kt[base:base + 32]
            w = _pack(jnp.concatenate([w, w, w, w], axis=0).T)
            ext = jnp.concatenate([carry_s[h], w], axis=0)
            carry_s[h] = w[CH // 2 - 48:]
            n = CH // 2
            ka_s[h, rows, :] = jnp.where(
                lane < 64, jnp.where(lane < 32, ext[0:n], ext[16:n + 16]),
                jnp.where(lane < 96, ext[32:n + 32], ext[48:n + 48]))
        q = _pack((_dot(wa_s[0:D, :], x) * QSCALE).astype(bf16))
        r16 = jax.lax.broadcasted_iota(i32, (16, CH), 0)
        for h in range(H):
            base = 16 * ((DH * h) // 16)
            qo = (DH * h - base) // 2
            w = jnp.where((r16 >= qo) & (r16 < qo + 9), q[base // 2:base // 2 + 16], 0)
            for t in range(TPC):
                qta_s[c * TPC + t, h] = w[:, t * T:(t + 1) * T]
        v = _dot(wa_s[2 * D:3 * D, :], x).astype(bf16).astype(f32)
        r24 = jax.lax.broadcasted_iota(i32, (24, CH), 0)
        for h in range(H):
            R = 8 * ((DH * h) // 8)
            o = DH * h - R
            w = jnp.where((r24 >= o) & (r24 < o + DH), v[R:R + 24],
                          jnp.where(r24 == (o + DH) % 24, 1.0, 0.0))
            for t in range(TPC):
                vta_s[c * TPC + t, h] = w[:, t * T:(t + 1) * T]
        return 0
    carry_s[...] = jnp.zeros(carry_s.shape, i32)
    jax.lax.fori_loop(0, NCH, aproj_body, 0)

    k0f = _unpack(kb_s[0, V0 // 2:S // 2, :]).astype(f32)
    for d in range(DH):
        kbc_s[d] = jnp.broadcast_to(k0f[:, d:d + 1], (RV, T))
    z_s[0] = 0
    zz = z_s[0]

    rr = jax.lax.broadcasted_iota(i32, (T, T), 0)
    cc = jax.lax.broadcasted_iota(i32, (T, T), 1)

    def b_step(jn, h, hn, buf, m_cur, do_pv=True):
        w0 = 8 * ((9 * hn) // 8)
        ko = (DH * hn - 2 * w0) // 2
        r64 = jax.lax.broadcasted_iota(i32, (64, T), 0)
        qt = _unpack(jnp.where(r64 < 16, qtb_s[jn, w0:w0 + 64, :], 0))
        qrows = [jnp.broadcast_to(qf_s[jn, DH * hn + d:DH * hn + d + 1, :], (8, T)) for d in range(DH)]
        o = h % 4
        mx = None
        acc = None
        done = 0
        for t in range(NJ):
            lo, hi = t * T, (t + 1) * T
            if do_pv:
                parts = []
                if lo < V0:
                    parts.append(sb_s[buf, lo:min(hi, V0), :])
                if hi > V0:
                    parts.append(vb_s[zz + h % 4, max(lo, V0) - V0:hi - V0, :])
                sc = parts[0] if len(parts) == 1 else jnp.concatenate(parts, axis=0)
            if lo < V0:
                h2 = min(hi, V0)
                s = _dot(_unpack(kb_s[ko, lo // 2:h2 // 2, :]), qt)
                sb_s[buf, lo:h2, :] = s
                mt = jnp.max(s.reshape((h2 - lo) // 8, 8, T), axis=0)
                mx = mt if mx is None else jnp.maximum(mx, mt)
            while done < -(-NVV * (t + 1) // NJ):
                prs = [kbc_s[d, done * 8:(done + 1) * 8, :] * qrows[d] for d in range(DH)]
                hs = prs[:NACC]
                for d in range(NACC, DH):
                    hs[d % NACC] = hs[d % NACC] + prs[d]
                a = hs[0]
                for x_ in hs[1:]:
                    a = a + x_
                vb_s[zz + hn % 4, done * 8:(done + 1) * 8, :] = a
                mx = a if mx is None else jnp.maximum(mx, a)
                done += 1
            if do_pv:
                p = jnp.exp2(sc - m_cur).astype(bf16)
                d_ = _dot(vtb_s[o, t], p)
                acc = d_ if acc is None else acc + d_
        m_new = jnp.max(mx, axis=0, keepdims=True)
        if not do_pv:
            return m_new, None
        dr = (DH + 2 * o) % 24
        inv = 1.0 / acc[dr:dr + 1, :]
        r = jax.lax.broadcasted_iota(i32, (24, T), 0)
        res = jnp.where((r >= 2 * o) & (r < 2 * o + DH), acc * inv, 0.0)
        return m_new, res

    ms = tuple(b_step(0, 0, u, u, None, do_pv=False)[0] for u in range(2))

    def b_body(j, ms):
        ms = list(ms)
        jn1 = jnp.minimum(j + 1, NJ - 1)
        parts = []
        for h in range(H):
            hn = (h + 2) % H
            jn = j if h + 2 < H else jn1
            ms[h % 2], res = b_step(jn, h, hn, h % 2, ms[h % 2])
            parts.append(res)
            if h % 4 == 3:
                G = h // 4
                otb_s[j, 72 * G:72 * G + 72, :] = _merge4(parts)
                parts = []
        return tuple(ms)
    jax.lax.fori_loop(0, NJ, b_body, ms)

    cp_awo.wait()
    cp_bwo.wait()
    woa_s[...] = awo_s[...].T
    wob_s[...] = bwo_s[...].T

    bias_s[0:T, :] = jnp.where(cc >= rr, 0.0, NEG)
    bias_s[T:T + 32, :] = jnp.where(rr > (cc & 31), 0.0, NEG)[0:32]
    bias_s[T + 32:T + 64, :] = jnp.where(rr <= (cc & 31), 0.0, NEG)[0:32]

    def a_step(cur, h, nxt, hn, buf, m_cur):
        o = DH * h - 8 * ((DH * h) // 8)
        dr = (o + DH) % 24
        l16 = jax.lax.broadcasted_iota(i32, (16, T), 1)
        l8 = jax.lax.broadcasted_iota(i32, (8, T), 1)

        def krows(w0, n):
            w0 = w0 if isinstance(w0, int) else pl.multiple_of(w0, 8)
            return ka_s[hn, pl.ds(w0, n), :]

        def plain_scores(jq, kt):
            q = jnp.concatenate([jnp.zeros((48, T), i32), qta_s[jq, hn]], axis=0)
            return _dot(_unpack(krows(kt * 64, 64)), _unpack(q))

        def by_group(srcs):
            srcs = [0 if x is None else x for x in srcs]
            out = srcs[3]
            for g in (2, 1, 0):
                if isinstance(srcs[g], int) and isinstance(srcs[g + 1], int):
                    continue
                out = jnp.where(l8 < 32 * (g + 1), srcs[g], out)
            return out

        def sheared_scores(jq):
            w = qta_s[jq, hn]
            q = jnp.concatenate(
                [jnp.where(l16 < 32, w, 0), jnp.where(l16 < 32, 0, jnp.where(l16 < 64, w, 0)),
                 jnp.where(l16 < 64, 0, jnp.where(l16 < 96, w, 0)), jnp.where(l16 < 96, 0, w)], axis=0)
            lo = krows((jq - 2) * 64 + 48, 64)
            hi = krows((jq - 1) * 64 + 48 + 16, 64)
            blocks = [lo[0:16]]
            for b in range(2, 8):
                blocks.append(jnp.where(l8 < 32 * ((7 - b) // 2 + 1), lo[8 * b:8 * b + 8], hi[8 * b - 16:8 * b - 8]))
            blocks.append(hi[48:64])
            s = _dot(_unpack(jnp.concatenate(blocks, axis=0)), _unpack(q))
            return jnp.concatenate([s[0:32] + bias_s[T:T + 32, :], s[32:128],
                                    s[128:160] + bias_s[T + 32:T + 64, :]], axis=0)

        def colmax(s):
            return jnp.max(s.reshape(s.shape[0] // 8, 8, T), axis=0)

        def pv(kt, p):
            return _dot(vta_s[kt, h], p)

        def finish(a):
            a = a * (1.0 / a[dr:dr + 1, :])
            b0 = 8 * (dr // 8)
            r8 = jax.lax.broadcasted_iota(i32, (8, T), 0)
            blk = jnp.where(r8 == dr - b0, 0.0, a[b0:b0 + 8])
            return jnp.concatenate([p for p in (a[0:b0], blk, a[b0 + 8:24]) if p.shape[0]], axis=0)

        def prob(s, m):
            return jnp.exp2(s - m).astype(bf16)

        sc = None
        if cur is not None:
            sizes = (T, T, T) if cur[1] else (160, T)
            sc, r0 = [], 0
            for n in sizes:
                sc.append(sa_s[buf, r0:r0 + n, :])
                r0 += n
        jn, first_n = nxt
        if first_n:
            new = [plain_scores(0, 0) + bias_s[0:T, :], plain_scores(1, 0),
                   plain_scores(1, 1) + bias_s[0:T, :]]
            mx = [colmax(new[0]), jnp.maximum(colmax(new[1]), colmax(new[2]))]
        else:
            new = [sheared_scores(jn), plain_scores(jn, jn - 1)]
            mx = [jnp.maximum(colmax(new[0]), colmax(new[1]))]
        r0 = 0
        for v in new:
            sa_s[buf, r0:r0 + v.shape[0], :] = v
            r0 += v.shape[0]
        m_new = [jnp.max(m, axis=0, keepdims=True) for m in mx]
        if cur is None:
            return m_new, None
        j, first = cur
        if first:
            res = [finish(pv(0, prob(sc[0], m_cur[0]))),
                   finish(pv(0, prob(sc[1], m_cur[1])) + pv(1, prob(sc[2], m_cur[1])))]
        else:
            pw = _pack(prob(sc[0], m_cur[0]))
            pb = [pw[8 * b:8 * b + 8] for b in range(10)]
            trail = jnp.concatenate(
                [by_group([pb[b - 2 * g] if b >= 2 * g else None for g in range(4)]) for b in range(8)],
                axis=0)
            diag = jnp.concatenate(
                [by_group([pb[b + 8 - 2 * g] if b < 2 * (g + 1) else None for g in range(4)])
                 for b in range(8)], axis=0)
            res = [finish(pv(j, _unpack(diag)) + pv(j - 2, _unpack(trail))
                          + pv(j - 1, prob(sc[1], m_cur[0])))]
        return m_new, res

    def out_tile(j):
        ra = _dot(woa_s[...], ota_s[j].astype(bf16))
        rb = _dot(wob_s[...], otb_s[j].astype(bf16))
        out_s[j] = jnp.concatenate([ra.astype(bf16), rb.astype(bf16)], axis=0).T
        r0 = j * T if isinstance(j, int) else pl.multiple_of(j * T, T)
        pltpu.make_async_copy(out_s.at[j], out_hbm.at[pl.ds(r0, T), :], osem.at[j]).start()

    def a_sweep(cur_fn, nxt_fn, ms):
        jq0 = cur_fn(0)[0]
        ms = list(ms)
        parts = None
        for h in range(H):
            hn = (h + NBA) % H
            ms[h % NBA], res = a_step(cur_fn(h), h, nxt_fn(h), hn, h % NBA, ms[h % NBA])
            parts = [[r] for r in res] if h % 4 == 0 else [p + [r] for p, r in zip(parts, res)]
            if h % 4 == 3:
                G = h // 4
                for gi, p in enumerate(parts):
                    ota_s[jq0 + gi, 72 * G:72 * G + 72, :] = _merge4(p)
        return ms

    ms = [a_step(None, 0, (0, True), u, u, None)[0] for u in range(NBA)]
    ms = a_sweep(lambda h: (0, True),
                 lambda h: (0, True) if h + NBA < H else (2, False), ms)
    out_tile(0)

    def a_one(j, ms):
        jn1 = jnp.minimum(j + 1, NJ - 1)
        out_tile(j - 1)
        return a_sweep(lambda h: (j, False),
                       lambda h: (j if h + NBA < H else jn1, False), [list(m) for m in ms])

    def a_body(i, ms):
        ms = a_one(2 * i, ms)
        ms = a_one(2 * i + 1, ms)
        return tuple(tuple(m) for m in ms)
    jax.lax.fori_loop(1, NJ // 2, a_body, tuple(tuple(m) for m in ms))
    out_tile(NJ - 1)

    for j in range(NJ):
        pltpu.make_async_copy(out_s.at[j], out_hbm.at[pl.ds(j * T, T), :], osem.at[j]).wait()


@jax.jit
def pallas_concat_heads__sliding_block__grouped_kv_mqa__prompt_kernel(
    A_x: jax.Array,
    A_wqkv: jax.Array,
    A_wo: jax.Array,
    B_x: jax.Array,
    B_wq: jax.Array,
    B_wk: jax.Array,
    B_wv: jax.Array,
    B_wo: jax.Array,
):
    scratch = [
        pltpu.VMEM((NCH, D, CH), bf16),
        pltpu.VMEM((NCH, D, CH), bf16),
        pltpu.VMEM((D, 3 * D), bf16),
        pltpu.VMEM((D, D), bf16),
        pltpu.VMEM((D, D), bf16),
        pltpu.VMEM((DH, D), bf16),
        pltpu.VMEM((DH, D), bf16),
        pltpu.VMEM((D, D), bf16),
        pltpu.VMEM((3 * D, D), bf16),
        pltpu.VMEM((D + 64, D), bf16),
        pltpu.VMEM((NJ, H, 16, T), i32),
        pltpu.VMEM((NJ, QW, T), i32),
        pltpu.VMEM((H, S // 2, T), i32),
        pltpu.VMEM((NJ, H, 24, T), f32),
        pltpu.VMEM((8, S // 2, T), i32),
        pltpu.VMEM((4, NJ, 24, T), f32),
        pltpu.VMEM((2, S, T), f32),
        pltpu.VMEM((NBA, 3 * T, T), f32),
        pltpu.VMEM((NJ, D, T), f32),
        pltpu.VMEM((NJ, D, T), f32),
        pltpu.VMEM((D, D), bf16),
        pltpu.VMEM((D, D), bf16),
        pltpu.VMEM((NJ, T, 2 * D), bf16),
        pltpu.VMEM((H, 48, T), i32),
        pltpu.VMEM((T + 64, T), f32),
        pltpu.VMEM((NJ, D, T), f32),
        pltpu.VMEM((DH, RV, T), f32),
        pltpu.VMEM((4, RV, T), f32),
        pltpu.SMEM((1,), i32),
        pltpu.SemaphoreType.DMA((6 + 2 * NCH,)),
        pltpu.SemaphoreType.DMA((NJ,)),
    ]
    anyspec = pl.BlockSpec(memory_space=pl.ANY)
    out = pl.pallas_call(
        _kernel,
        out_shape=jax.ShapeDtypeStruct((S, 2 * D), bf16),
        in_specs=[anyspec] * 8,
        out_specs=anyspec,
        scratch_shapes=scratch,
        compiler_params=pltpu.CompilerParams(vmem_limit_bytes=100 * 1024 * 1024),
        name="fused_attn_pair",
    )(A_x.reshape(S, D).T, A_wqkv, A_wo, B_x.reshape(S, D).T, B_wq, B_wk.T, B_wv.T, B_wo)
    return out.reshape(1, S, 2 * D)
```
